```python
import os as _os
_os.environ.setdefault("JAX_PLATFORMS", "cpu")
import jax
import jax.numpy as jnp

def _softmax(x, axis=-1):
    return jax.nn.softmax(x, axis=axis)
def _gelu(x):
    return jax.nn.gelu(x, approximate=True)
def _silu(x):
    return jax.nn.silu(x)
def _sigmoid(x):
    return jax.nn.sigmoid(x)
def _layernorm(x, axis=-1, eps=1e-5):
    m = jnp.mean(x, axis=axis, keepdims=True)
    v = jnp.var(x, axis=axis, keepdims=True)
    return (x - m) / jnp.sqrt(v + eps)
def _scatter_add(tgt, idx, src, axis=0):
    return tgt.at[idx].add(src)
def _segment_sum(src, seg, n):
    return jax.ops.segment_sum(src, seg, n)
class _Rng:
    def __init__(self, key):
        self._k = key
    def _next(self):
        self._k, sub = jax.random.split(self._k)
        return sub
    def normal(self, shape):
        return jax.random.normal(self._next(), shape, dtype=jnp.bfloat16)
    def randint(self, lo, hi, shape):
        return jax.random.randint(self._next(), shape, lo, hi, dtype=jnp.int32)
    def uniform(self, shape, lo=0.0, hi=1.0):
        return jax.random.uniform(self._next(), shape, jnp.bfloat16, lo, hi)
    def permutation(self, n):
        return jax.random.permutation(self._next(), n)


kernel_name = 'parallel_sum__ssm_conv_s4__mixer_channel_mlp__prompt'

def setup_inputs():
    _rng = _Rng(jax.random.key(int.from_bytes(__import__("os").urandom(4), "little")))
    _w = (lambda a: (lambda t: t.astype(jnp.bfloat16) if jnp.issubdtype(t.dtype, jnp.floating) else t)(jnp.asarray(a)))
    def _A_setup():
        B, L, D, N = 1, 2048, 512, 128
        A_re = -jnp.exp((lambda *s: _rng.normal(s) * 0.1)(D, N))
        A_im = jnp.pi * (lambda *s: _rng.normal(s) * 0.1)(D, N)
        B_re = (lambda *s: _rng.normal(s) * 0.1)(D, N)
        B_im = (lambda *s: _rng.normal(s) * 0.1)(D, N)
        C_re = (lambda *s: _rng.normal(s) * 0.1)(D, N)
        C_im = (lambda *s: _rng.normal(s) * 0.1)(D, N)
        log_dt = (lambda *s: _rng.normal(s) * 0.1)(D) * 0.5 - 4.0
        Dskip = (lambda *s: _rng.normal(s) * 0.05)(D)
        return {
            "u": _w((lambda *s: _rng.normal(s) * 0.05)(B, L, D)),
            "A_re": _w(A_re),
            "A_im": _w(A_im),
            "B_re": _w(B_re),
            "B_im": _w(B_im),
            "C_re": _w(C_re),
            "C_im": _w(C_im),
            "log_dt": _w(log_dt),
            "Dskip": _w(Dskip),
        }
    _A_in = _A_setup()

    def _B_setup():
        B, S, D, F = 1, 2048, 512, 1792
        return {
            "x": _w((lambda *s: _rng.normal(s) * 0.05)(B, S, D)),
            "w1": _w((lambda *s: _rng.normal(s) * 0.2)(D, F) * (D ** -0.5)),
            "b1": _w((lambda *s: _rng.normal(s) * 0.2)(F)),
            "w2": _w((lambda *s: _rng.normal(s) * 0.2)(F, D) * (F ** -0.5)),
            "b2": _w((lambda *s: _rng.normal(s) * 0.05)(D)),
        }
    _B_in = _B_setup()

    return {
        "A_u": _A_in["u"],
        "A_A_re": _A_in["A_re"],
        "A_A_im": _A_in["A_im"],
        "A_B_re": _A_in["B_re"],
        "A_B_im": _A_in["B_im"],
        "A_C_re": _A_in["C_re"],
        "A_C_im": _A_in["C_im"],
        "A_log_dt": _A_in["log_dt"],
        "A_Dskip": _A_in["Dskip"],
        "B_x": _B_in["x"],
        "B_w1": _B_in["w1"],
        "B_b1": _B_in["b1"],
        "B_w2": _B_in["w2"],
        "B_b2": _B_in["b2"],
    }

def reference(A_u, A_A_re, A_A_im, A_B_re, A_B_im, A_C_re, A_C_im, A_log_dt, A_Dskip, B_x, B_w1, B_b1, B_w2, B_b2):
    def _A_ref(u, A_re, A_im, B_re, B_im, C_re, C_im, log_dt, Dskip):
        Bsz, L, D = u.shape
        dt = jnp.exp(log_dt)[:, None]
        A = A_re + 1j * A_im
        Bc = B_re + 1j * B_im
        Cc = C_re + 1j * C_im
        logdA = dt * A
        dB = dt * Bc
        l = (lambda x, dt: x.astype(dt))(jnp.arange(L), A_re.dtype)
        P = jnp.exp(logdA[:, :, None] * l[None, None, :])
        K = jnp.einsum("dn,dnl,dn->dl", Cc, P, dB).real
        L2 = 2 * L
        Kp = jnp.pad(K, ((0, 0), (0, L)))
        up = (lambda x, *d: x.transpose(*d))(u, 0, 2, 1)
        up = jnp.pad(up, ((0, 0), (0, 0), (0, L)))
        Kf = (lambda x, axes=(-2,-1): jnp.fft.rfft2(x.astype(jnp.float32), axes=axes))(Kp[:, None, :], axes=(-2, -1))
        Uf = (lambda x, axes=(-2,-1): jnp.fft.rfft2(x.astype(jnp.float32), axes=axes))(up[:, :, None, :], axes=(-2, -1))
        Yf = Uf * Kf[None, :, :, :]
        y = (lambda x, s, axes=(-2,-1): jnp.fft.irfft2(x, s=s, axes=axes).astype(jnp.bfloat16))(Yf, (1, L2), axes=(-2, -1))[:, :, 0, :L]
        y = (lambda x, *d: x.transpose(*d))(y, 0, 2, 1) + u * Dskip[None, None, :]
        return y

    def _B_ref(x, w1, b1, w2, b2):
        y = _layernorm(x, axis=-1)
        h = _gelu(jnp.einsum("bsd,df->bsf", y, w1) + b1)
        return jnp.einsum("bsf,fd->bsd", h, w2) + b2

    x = A_u
    xn = _layernorm(x, axis=-1)
    return x + _A_ref(xn, A_A_re, A_A_im, A_B_re, A_B_im, A_C_re, A_C_im, A_log_dt, A_Dskip) + _B_ref(xn, B_w1, B_b1, B_w2, B_b2)
```

```python
import functools, math
import numpy as np
import jax, jax.numpy as jnp
from jax.experimental import pallas as pl
from jax.experimental.pallas import tpu as pltpu

L, D, N, F = 2048, 512, 128, 1792
NF = 4096
N1, N2 = 64, 64
NA = L // N2
NK1 = N1 // 2 + 1
f32, bf16 = jnp.float32, jnp.bfloat16
RUN = 16
SEGS = ((1, 16, 0), (2, 8, 256), (4, 8, 384), (8, 8, 512))
NE = 641

def _dft_mats():
    b = np.arange(N2)
    G = np.zeros((NK1, 2 * N2, 2 * N2), np.float64)
    Gi = np.zeros((NK1, 2 * N2, 2 * N2), np.float64)
    for k1 in range(NK1):
        ang = -2 * np.pi * (np.outer(b, b) / N2 + (b * k1 / NF)[None, :])
        C, S = np.cos(ang), np.sin(ang)
        G[k1] = np.block([[C, -S], [S, C]])
        ang = 2 * np.pi * (np.outer(b, b) / N2 + (b * k1 / NF)[:, None])
        C, S = np.cos(ang) / NF, np.sin(ang) / NF
        Gi[k1] = np.block([[C, -S], [S, C]])
    return G, Gi

def _add(a, b):
    return (a[0] + b[0], a[1] if b[1] is None else (b[1] if a[1] is None else a[1] + b[1]))
def _sub(a, b):
    return (a[0] - b[0], a[1] if b[1] is None else ((-b[1]) if a[1] is None else a[1] - b[1]))
def _mulc(a, c, s):
    ar, ai = a
    def sc(v, k):
        if v is None or k == 0.0: return None
        if k == 1.0: return v
        if k == -1.0: return -v
        return v * k
    def pm(u, v, sign):
        if u is None: return v if (v is None or sign > 0) else -v
        if v is None: return u
        return u + v if sign > 0 else u - v
    re = pm(sc(ar, c), sc(ai, s), -1)
    im = pm(sc(ar, s), sc(ai, c), +1)
    if re is None: re = jnp.zeros_like(ar)
    return (re, im)
def _snap(v):
    r = round(v)
    return float(r) if abs(v - r) < 1e-12 else v
def _fft(xs, sign):
    n = len(xs)
    if n == 1: return xs
    h = n // 2
    a = [_add(xs[i], xs[i + h]) for i in range(h)]
    b = [_mulc(_sub(xs[i], xs[i + h]), _snap(math.cos(2 * math.pi * i / n)), _snap(sign * math.sin(2 * math.pi * i / n))) for i in range(h)]
    E, O = _fft(a, sign), _fft(b, sign)
    out = [None] * n
    for k in range(h):
        out[2 * k], out[2 * k + 1] = E[k], O[k]
    return out

def _ln(xb):
    xf = xb.astype(f32)
    mean = jnp.mean(xf, axis=-1, keepdims=True)
    var = jnp.mean(jnp.square(xf - mean), axis=-1, keepdims=True)
    m = mean.astype(bf16).astype(f32)
    v = var.astype(bf16).astype(f32)
    xc = (xf - m).astype(bf16).astype(f32)
    s = jnp.sqrt((v + 1e-5).astype(bf16).astype(f32)).astype(bf16).astype(f32)
    return (xc / s).astype(bf16)

def _fwd_stage1(src_ref, z_ref):
    def blk(i, carry):
        r0 = pl.multiple_of((i // 4) * 8, 8)
        c0 = pl.multiple_of((i % 4) * 128, 128)
        X = [src_ref[pl.ds(N2 * a + r0, 8), pl.ds(c0, 128)].astype(f32) for a in range(NA)]
        ev = _fft([(X[a], None) for a in range(NA)], -1)
        od = _fft([_mulc((X[a], None), _snap(math.cos(2 * math.pi * a / N1)), _snap(-math.sin(2 * math.pi * a / N1))) for a in range(NA)], -1)
        for k1 in range(NK1):
            re, im = ev[k1 // 2] if k1 % 2 == 0 else od[k1 // 2]
            z_ref[k1, pl.ds(r0, 8), pl.ds(c0, 128)] = re
            z_ref[k1, pl.ds(N2 + r0, 8), pl.ds(c0, 128)] = jnp.zeros_like(re) if im is None else im
        return carry
    jax.lax.fori_loop(0, 32, blk, 0)

def _inv_stage1(y_ref, dst_ref):
    def blk(i, carry):
        r0 = pl.multiple_of((i // 4) * 8, 8)
        c0 = pl.multiple_of((i % 4) * 128, 128)
        c = [(y_ref[k1, pl.ds(r0, 8), pl.ds(c0, 128)], y_ref[k1, pl.ds(N2 + r0, 8), pl.ds(c0, 128)]) for k1 in range(NK1)]
        def full(k):
            return c[k] if k <= N1 // 2 else (c[N1 - k][0], -c[N1 - k][1])
        E = _fft([full(2 * j) for j in range(32)], +1)
        O = _fft([full(2 * j + 1) for j in range(32)], +1)
        for a in range(NA):
            o = _mulc(O[a], _snap(math.cos(2 * math.pi * a / N1)), _snap(math.sin(2 * math.pi * a / N1)))
            dst_ref[pl.ds(N2 * a + r0, 8), pl.ds(c0, 128)] = E[a][0] + o[0]
        return carry
    jax.lax.fori_loop(0, 32, blk, 0)

def kernel(x_ref, are_ref, aim_ref, bre_ref, bim_ref, cre_ref, cim_ref, ldt_ref, dsk_ref,
           w1_ref, b1_ref, w2_ref, b2_ref, g_ref, gi_ref, o_ref,
           xn_ref, tab_ref, kp_ref, k_ref, zx_ref, zk_ref, y_ref, yt_ref, ob_ref):
    xn_ref[...] = _ln(x_ref[...])

    dt = jnp.exp(ldt_ref[...].astype(f32)).astype(bf16).astype(f32)
    ar = are_ref[...].astype(f32).T * dt
    ai = aim_ref[...].astype(f32).T * dt
    dbr = bre_ref[...].astype(f32).T * dt
    dbi = bim_ref[...].astype(f32).T * dt
    cr = cre_ref[...].astype(f32).T
    ci = cim_ref[...].astype(f32).T
    tab_ref[24] = cr * dbr - ci * dbi
    tab_ref[25] = cr * dbi + ci * dbr
    mag = jnp.exp(ar)
    pw = [(mag * jnp.cos(ai), mag * jnp.sin(ai), mag * mag)]
    for j in range(7):
        wr, wi, m2 = pw[-1]
        pw.append((wr * wr - wi * wi, 2.0 * (wr * wi), m2 * m2))
    for si, (h, _, _) in enumerate(SEGS):
        wr, wi, m2 = pw[si]
        tab_ref[6 * si + 0] = wr
        tab_ref[6 * si + 1] = wi
        tab_ref[6 * si + 2] = wr * 2.0
        tab_ref[6 * si + 3] = m2
        tab_ref[6 * si + 4] = pw[si + 4][0]
        tab_ref[6 * si + 5] = pw[si + 4][1]
    kp_ref[...] = jnp.zeros_like(kp_ref)

    def kgen(sb):
        rows = pl.ds(pl.multiple_of(sb * 8, 8), 8)
        zr, zi = tab_ref[24, rows, :], tab_ref[25, rows, :]
        for si, (h, nruns, base) in enumerate(SEGS):
            for rr in range(nruns):
                wr, wi = tab_ref[6 * si + 0, rows, :], tab_ref[6 * si + 1, rows, :]
                p, q = tab_ref[6 * si + 2, rows, :], tab_ref[6 * si + 3, rows, :]
                m0 = base + rr * RUN
                r0 = zr
                r1 = zr * wr - zi * wi
                kp_ref[m0] += r0
                kp_ref[m0 + 1] += r1
                for st in range(2, RUN):
                    r2 = p * r1 - q * r0
                    kp_ref[m0 + st] += r2
                    r0, r1 = r1, r2
                Wr, Wi = tab_ref[6 * si + 4, rows, :], tab_ref[6 * si + 5, rows, :]
                zr, zi = zr * Wr - zi * Wi, zr * Wi + zi * Wr
        kp_ref[NE - 1] += zr

    TM = 256
    def mlp(i, carry):
        kgen(2 * i)
        kgen(2 * i + 1)
        rows = pl.ds(pl.multiple_of(i * TM, TM), TM)
        xn = xn_ref[rows, :]
        y2 = _ln(xn)
        h = jnp.dot(y2, w1_ref[...], preferred_element_type=f32).astype(bf16).astype(f32)
        h = (h + b1_ref[...].astype(f32)).astype(bf16).astype(f32)
        h = jax.nn.gelu(h, approximate=True).astype(bf16)
        ob = jnp.dot(h, w2_ref[...], preferred_element_type=f32).astype(bf16).astype(f32)
        ob_ref[rows, :] = (ob + b2_ref[...].astype(f32)).astype(bf16)
        return carry
    jax.lax.fori_loop(0, L // TM, mlp, 0)

    kt = jnp.sum(kp_ref[...], axis=1)
    k_ref[0:256, :] = kt[0:256]
    for (h, _, base) in SEGS[1:]:
        s0 = 128 * h
        T = kt[base:base + 136]
        Rr = jnp.broadcast_to(T[:, None, :], (136, h, D)).reshape(136 * h, D)
        up = Rr[h // 2: h // 2 + s0]
        dn = Rr[h // 2 - 1: h // 2 - 1 + s0]
        u = jax.lax.broadcasted_iota(jnp.int32, (s0, D), 0)
        tie_dn = jnp.logical_and(u % h == h // 2, ((u + h // 2) // h) % 2 == 1)
        k_ref[s0:2 * s0, :] = jnp.where(tie_dn, dn, up)

    _fwd_stage1(xn_ref, zx_ref)
    _fwd_stage1(k_ref, zk_ref)
    def k1_body(k1, carry):
        g = g_ref[k1]
        xh = jnp.dot(g, zx_ref[k1].astype(bf16), preferred_element_type=f32)
        kh = jnp.dot(g, zk_ref[k1].astype(bf16), preferred_element_type=f32)
        xr, xi, kr, ki = xh[:N2], xh[N2:], kh[:N2], kh[N2:]
        yh = jnp.concatenate([xr * kr - xi * ki, xr * ki + xi * kr], axis=0).astype(bf16)
        y_ref[k1] = jnp.dot(gi_ref[k1], yh, preferred_element_type=f32)
        return carry
    jax.lax.fori_loop(0, NK1, k1_body, 0)
    _inv_stage1(y_ref, yt_ref)

    x = x_ref[...]
    xn = xn_ref[...]
    sk = (xn.astype(f32) * dsk_ref[...].astype(f32)).astype(bf16).astype(f32)
    ya = (yt_ref[...].astype(bf16).astype(f32) + sk).astype(bf16).astype(f32)
    o = (x.astype(f32) + ya).astype(bf16).astype(f32)
    o_ref[...] = (o + ob_ref[...].astype(f32)).astype(bf16)


_G, _GI = _dft_mats()
_G = _G.astype(np.float32)
_GI = _GI.astype(np.float32)


@jax.jit
def pallas_parallel_sum__ssm_conv_s4__mixer_channel_mlp__prompt_kernel(
    A_u: jax.Array,
    A_A_re: jax.Array,
    A_A_im: jax.Array,
    A_B_re: jax.Array,
    A_B_im: jax.Array,
    A_C_re: jax.Array,
    A_C_im: jax.Array,
    A_log_dt: jax.Array,
    A_Dskip: jax.Array,
    B_x: jax.Array,
    B_w1: jax.Array,
    B_b1: jax.Array,
    B_w2: jax.Array,
    B_b2: jax.Array,
):
    del B_x
    out = pl.pallas_call(
        kernel,
        out_shape=jax.ShapeDtypeStruct((L, D), bf16),
        scratch_shapes=[
            pltpu.VMEM((L, D), bf16),
            pltpu.VMEM((26, N, D), f32),
            pltpu.VMEM((648, 8, D), f32),
            pltpu.VMEM((L, D), f32),
            pltpu.VMEM((NK1, 128, D), f32),
            pltpu.VMEM((NK1, 128, D), f32),
            pltpu.VMEM((NK1, 128, D), f32),
            pltpu.VMEM((L, D), f32),
            pltpu.VMEM((L, D), bf16),
        ],
        compiler_params=pltpu.CompilerParams(vmem_limit_bytes=110 * 1024 * 1024),
    )(A_u.reshape(L, D), A_A_re, A_A_im, A_B_re, A_B_im, A_C_re, A_C_im,
      A_log_dt.reshape(1, D), A_Dskip.reshape(1, D), B_w1, B_b1.reshape(1, F), B_w2,
      B_b2.reshape(1, D), jnp.asarray(_G, dtype=bf16), jnp.asarray(_GI, dtype=bf16))
    return out.reshape(1, L, D)
```
